```python
import os as _os
_os.environ.setdefault("JAX_PLATFORMS", "cpu")
import jax
import jax.numpy as jnp

def _softmax(x, axis=-1):
    return jax.nn.softmax(x, axis=axis)
def _gelu(x):
    return jax.nn.gelu(x, approximate=True)
def _silu(x):
    return jax.nn.silu(x)
def _sigmoid(x):
    return jax.nn.sigmoid(x)
def _layernorm(x, axis=-1, eps=1e-5):
    m = jnp.mean(x, axis=axis, keepdims=True)
    v = jnp.var(x, axis=axis, keepdims=True)
    return (x - m) / jnp.sqrt(v + eps)
def _scatter_add(tgt, idx, src, axis=0):
    return tgt.at[idx].add(src)
def _segment_sum(src, seg, n):
    return jax.ops.segment_sum(src, seg, n)
class _Rng:
    def __init__(self, key):
        self._k = key
    def _next(self):
        self._k, sub = jax.random.split(self._k)
        return sub
    def normal(self, shape):
        return jax.random.normal(self._next(), shape, dtype=jnp.bfloat16)
    def randint(self, lo, hi, shape):
        return jax.random.randint(self._next(), shape, lo, hi, dtype=jnp.int32)
    def uniform(self, shape, lo=0.0, hi=1.0):
        return jax.random.uniform(self._next(), shape, jnp.bfloat16, lo, hi)
    def permutation(self, n):
        return jax.random.permutation(self._next(), n)


kernel_name = 'standalone__gqa_softmax__near_ridge'

def setup_inputs():
    _rng = _Rng(jax.random.key(int.from_bytes(__import__("os").urandom(4), "little")))
    _w = (lambda a: (lambda t: t.astype(jnp.bfloat16) if jnp.issubdtype(t.dtype, jnp.floating) else t)(jnp.asarray(a)))
    B, Hq, Hkv, Sq, Sk, D = 8, 16, 8, 160, 2048, 256
    return {
        "q": _w((lambda *s: _rng.normal(s) * 0.05)(B, Hq, Sq, D)),
        "k": _w((lambda *s: _rng.normal(s) * 3.2)(B, Hkv, Sk, D)),
        "v": _w((lambda *s: _rng.normal(s) * 0.05)(B, Hkv, Sk, D)),
    }

def reference(q, k, v):
    B, Hq, Sq, D = q.shape
    Hkv = k.shape[1]
    rep = Hq // Hkv
    k = jnp.repeat(k, rep, axis=1)
    v = jnp.repeat(v, rep, axis=1)
    scale = D ** -0.5
    scores = jnp.einsum("bhqd,bhkd->bhqk", q, k) * scale
    p = _softmax(scores, axis=-1)
    return jnp.einsum("bhqk,bhkd->bhqd", p, v)
```

```python
import jax
import jax.numpy as jnp
import numpy as np
from jax import lax
import jax.experimental.pallas as pl
import jax.experimental.pallas.tpu as pltpu

_LOG2E = 1.4426950408889634
_CONTRACT_LAST = (((1,), (1,)), ((), ()))
_LANES = 128

_UNROLL = 9
_NBUF = 3
_CHUNK = 256
_NDMA = 2
_TIE = (1, 6, 7)


def _after(x, dep):
    z = lax.shift_right_arithmetic(
        lax.bitcast_convert_type(dep, jnp.int32) | np.int32(-(2**31)), np.int32(31)
    )
    return lax.bitcast_convert_type(
        lax.bitcast_convert_type(x, jnp.int32) & z, jnp.float32
    )


def _when(cond, fn):
    if isinstance(cond, (bool, np.bool_)):
        if cond:
            fn()
    else:
        pl.when(cond)(fn)


@jax.jit
def pallas_standalone__gqa_softmax__near_ridge_kernel(
    q: jax.Array,
    k: jax.Array,
    v: jax.Array,
):
    B, Hq, Sq, D = q.shape
    Hkv, Sk = k.shape[1], k.shape[2]
    M = (Hq // Hkv) * Sq
    N = B * Hkv
    exp_scale = (D**-0.5) * _LOG2E

    nbuf, chunk, ndma = _NBUF, _CHUNK, _NDMA
    nchunk = Sk // chunk
    piece = Sk // ndma
    unroll = min(_UNROLL, max(N - 1, 1))
    niter, tail = divmod(N - 1, unroll)
    assert Sk % (chunk * ndma) == 0 and chunk % _LANES == 0 and N >= nbuf
    assert unroll % nbuf == 0 or niter <= 1
    sem_k0, sem_v0 = nbuf, nbuf + nbuf * ndma

    def kernel_function(
        q_hbm, k_hbm, v_hbm, o_hbm,
        q_buf, k_buf, v_buf, o_buf, s_buf, m_buf, in_sems, out_sems,
    ):
        def q_copy(h, slot):
            return pltpu.make_async_copy(q_hbm.at[h], q_buf.at[slot], in_sems.at[slot])

        def k_copy(h, slot, i):
            rows = pl.ds(i * piece, piece)
            return pltpu.make_async_copy(
                k_hbm.at[h, rows], k_buf.at[slot, rows],
                in_sems.at[sem_k0 + slot * ndma + i],
            )

        def v_copy(h, slot, i):
            rows = pl.ds(i * piece, piece)
            return pltpu.make_async_copy(
                v_hbm.at[h, rows], v_buf.at[slot, rows],
                in_sems.at[sem_v0 + slot * ndma + i],
            )

        def o_copy(h, slot):
            return pltpu.make_async_copy(o_buf.at[slot], o_hbm.at[h], out_sems.at[slot])

        def fetch_qk(h, slot):
            q_copy(h, slot).start()
            for i in range(ndma):
                k_copy(h, slot, i).start()

        def fetch_v(h, slot):
            for i in range(ndma):
                v_copy(h, slot, i).start()

        class Scores:
            def __init__(self, h, slot):
                self.h, self.slot, self.q, self.running_max = h, slot, None, None

            def step(self, j):
                if (j * chunk) % piece == 0:
                    k_copy(self.h, self.slot, j * chunk // piece).wait()
                if j == 0:
                    q_copy(self.h, self.slot).wait()
                    self.q = q_buf[self.slot]
                keys = pl.ds(j * chunk, chunk)
                s = lax.dot_general(
                    self.q, k_buf[self.slot, keys, :], _CONTRACT_LAST,
                    preferred_element_type=jnp.float32,
                )
                s_buf[:, keys] = s
                mx = s[:, :_LANES]
                for u in range(1, chunk // _LANES):
                    mx = jnp.maximum(mx, s[:, u * _LANES:(u + 1) * _LANES])
                if self.running_max is not None:
                    mx = jnp.maximum(self.running_max, mx)
                self.running_max = mx
                if j == nchunk - 1:
                    row_max = jnp.max(mx, axis=-1, keepdims=True)
                    m_buf[...] = jnp.broadcast_to(row_max, (M, _LANES))

        class Attend:
            def __init__(self, h, slot, out_slot, prev, scores):
                self.h, self.slot, self.out_slot = h, slot, out_slot
                self.prev, self.scores = prev, scores
                self.m = self.row_sum = self.acc = self.inv = None
                self.p = {}

            def probs(self, j):
                if self.m is None:
                    self.m = m_buf[...]
                    if self.prev is not None:
                        inv = jnp.broadcast_to(self.prev.inv_sum(), (M, _LANES))
                        self.m = _after(self.m, inv)
                if j in _TIE and self.scores is not None:
                    self.m = _after(self.m, self.scores.running_max)
                s = s_buf[:, pl.ds(j * chunk, chunk)]
                ps = [
                    jnp.exp2((s[:, u * _LANES:(u + 1) * _LANES] - self.m) * exp_scale)
                    for u in range(chunk // _LANES)
                ]
                part = ps[0]
                for p in ps[1:]:
                    part = part + p
                self.row_sum = part if self.row_sum is None else self.row_sum + part
                self.p[j] = jnp.concatenate(ps, axis=1).astype(v_buf.dtype)

            def accumulate(self, j):
                if (j * chunk) % piece == 0:
                    v_copy(self.h, self.slot, j * chunk // piece).wait()
                o = jnp.dot(
                    self.p.pop(j), v_buf[self.slot, pl.ds(j * chunk, chunk), :],
                    preferred_element_type=jnp.float32,
                )
                self.acc = o if self.acc is None else self.acc + o

            def inv_sum(self):
                if self.inv is None:
                    self.inv = 1.0 / jnp.sum(self.row_sum, axis=-1, keepdims=True)
                return self.inv

            def finish(self):
                h, slot = self.h, self.out_slot
                _when(h >= unroll, lambda: o_copy(h - unroll, slot).wait())
                o_buf[slot] = (self.acc * self.inv_sum()).astype(o_buf.dtype)
                o_copy(h, slot).start()

        def stage(t, t_static, prev, do_scores=True):
            hv = t - 2 + nbuf
            _when(hv < N, lambda: fetch_v(hv, (t_static - 2 + nbuf) % nbuf))
            scores = None
            if do_scores:
                hk = t - 1 + nbuf
                _when(hk < N, lambda: fetch_qk(hk, (t_static - 1 + nbuf) % nbuf))
                scores = Scores(t, t_static % nbuf)
            attend = Attend(
                t - 1, (t_static - 1) % nbuf, (t_static - 1) % unroll, prev, scores
            )
            for j in range(nchunk):
                attend.probs(j)
                if do_scores:
                    scores.step(j)
                attend.accumulate(j)
            attend.finish()
            return attend

        def stages(t0, t0_static, n):
            prev = None
            for u in range(n):
                prev = stage(t0 + u, t0_static + u, prev)

        fetch_qk(0, 0)
        for h in range(1, nbuf - 1):
            q_copy(h, h).start()
            for i in range(ndma):
                k_copy(h, h, i).start()
                v_copy(h - 1, h - 1, i).start()
        fetch_qk(nbuf - 1, nbuf - 1)
        fetch_v(nbuf - 2, nbuf - 2)
        first = Scores(0, 0)
        for j in range(nchunk):
            first.step(j)

        def body(i, carry):
            stages(1 + i * unroll, 1, unroll)
            return carry

        lax.fori_loop(0, niter, body, 0)
        if tail:
            stages(1 + niter * unroll, 1 + niter * unroll, tail)

        stage(N, N, None, do_scores=False)
        for h in range(max(N - unroll, 0), N):
            o_copy(h, h % unroll).wait()

    out = pl.pallas_call(
        kernel_function,
        grid=(),
        in_specs=[pl.BlockSpec(memory_space=pl.ANY)] * 3,
        out_specs=pl.BlockSpec(memory_space=pl.ANY),
        out_shape=jax.ShapeDtypeStruct((N, M, D), q.dtype),
        scratch_shapes=[
            pltpu.VMEM((nbuf, M, D), q.dtype),
            pltpu.VMEM((nbuf, Sk, D), k.dtype),
            pltpu.VMEM((nbuf, Sk, D), v.dtype),
            pltpu.VMEM((unroll, M, D), q.dtype),
            pltpu.VMEM((M, Sk), jnp.float32),
            pltpu.VMEM((M, _LANES), jnp.float32),
            pltpu.SemaphoreType.DMA((nbuf + 2 * nbuf * ndma,)),
            pltpu.SemaphoreType.DMA((unroll,)),
        ],
        compiler_params=pltpu.CompilerParams(
            vmem_limit_bytes=64 * 1024 * 1024,
            flags={"XLA_TPU_RESCHEDULE_DMA_DONES": True},
        ),
    )(q.reshape(N, M, D), k.reshape(N, Sk, D), v.reshape(N, Sk, D))
    return out.reshape(B, Hq, Sq, D)
```
